```python
import os as _os
_os.environ.setdefault("JAX_PLATFORMS", "cpu")
import jax
import jax.numpy as jnp

def _softmax(x, axis=-1):
    return jax.nn.softmax(x, axis=axis)
def _gelu(x):
    return jax.nn.gelu(x, approximate=True)
def _silu(x):
    return jax.nn.silu(x)
def _sigmoid(x):
    return jax.nn.sigmoid(x)
def _layernorm(x, axis=-1, eps=1e-5):
    m = jnp.mean(x, axis=axis, keepdims=True)
    v = jnp.var(x, axis=axis, keepdims=True)
    return (x - m) / jnp.sqrt(v + eps)
def _scatter_add(tgt, idx, src, axis=0):
    return tgt.at[idx].add(src)
def _segment_sum(src, seg, n):
    return jax.ops.segment_sum(src, seg, n)
class _Rng:
    def __init__(self, key):
        self._k = key
    def _next(self):
        self._k, sub = jax.random.split(self._k)
        return sub
    def normal(self, shape):
        return jax.random.normal(self._next(), shape, dtype=jnp.bfloat16)
    def randint(self, lo, hi, shape):
        return jax.random.randint(self._next(), shape, lo, hi, dtype=jnp.int32)
    def uniform(self, shape, lo=0.0, hi=1.0):
        return jax.random.uniform(self._next(), shape, jnp.bfloat16, lo, hi)
    def permutation(self, n):
        return jax.random.permutation(self._next(), n)


kernel_name = 'standalone__gqa_block_cached__near_ridge'

def setup_inputs():
    _rng = _Rng(jax.random.key(int.from_bytes(__import__("os").urandom(4), "little")))
    _w = (lambda a: (lambda t: t.astype(jnp.bfloat16) if jnp.issubdtype(t.dtype, jnp.floating) else t)(jnp.asarray(a)))
    B, Sq, D = 16, 128, 576
    Hq, Hkv, Sk, Dh = 32, 16, 1024, 128
    assert Hq % Hkv == 0, (Hq, Hkv)
    return {
        "x": _w((lambda *s: _rng.normal(s) * 0.8)(B, Sq, D)),
        "k_cache": _w((lambda *s: _rng.normal(s) * 0.8)(B, Hkv, Sk, Dh)),
        "v_cache": _w((lambda *s: _rng.normal(s) * 0.05)(B, Hkv, Sk, Dh)),
        "wq": _w((lambda *s: _rng.normal(s) * 0.8)(D, Hq * Dh) * (D ** -0.5)),
        "wo": _w((lambda *s: _rng.normal(s) * 0.05)(Hq * Dh, D) * ((Hq * Dh) ** -0.5)),
    }

def reference(x, k_cache, v_cache, wq, wo):
    B, Sq, D = x.shape
    Hq, Dh = 32, 128
    Hkv = k_cache.shape[1]
    rep = Hq // Hkv
    q = (lambda x, *d: x.transpose(*d))((x @ wq).reshape(B, Sq, Hq, Dh), 0, 2, 1, 3)
    k = jnp.repeat(k_cache, rep, axis=1)
    v = jnp.repeat(v_cache, rep, axis=1)
    scores = jnp.einsum("bhqd,bhkd->bhqk", q, k) * (Dh ** -0.5)
    p = _softmax(scores, axis=-1)
    o = jnp.einsum("bhqk,bhkd->bhqd", p, v)
    return (lambda x, *d: x.transpose(*d))(o, 0, 2, 1, 3).reshape(B, Sq, Hq * Dh) @ wo
```

```python
import math

import jax
import jax.numpy as jnp
from jax import lax
import jax.experimental.pallas as pl
import jax.experimental.pallas.tpu as pltpu

_NT = (((1,), (1,)), ((), ()))

_SLAB = 32
_OP_CHUNKS = 2
_US = 4
_XG = 4
_GOUT = (8, 13, 15)


def _kernel(xT_hbm, k_hbm, v_hbm, wq_hbm, woT_hbm, o_hbm,
            xT_buf, x_buf, wq_buf, wo_buf, k_buf, v_buf, q_buf, p_buf, l_buf, o_buf, acc, ostage,
            x_sem, wq_sem, wo_sem, k_sem, v_sem, o_sem):
    bf16, f32, i32 = jnp.bfloat16, jnp.float32, jnp.int32
    B, D, Sq = xT_hbm.shape
    _, H, Sk, Dh = k_hbm.shape
    rep = wq_hbm.shape[1] // Dh // H
    M = rep * Sq
    NC = pl.cdiv(D, Dh)
    NG = B // _US
    OC = D // _OP_CHUNKS
    assert B & (B - 1) == 0 and B % _US == 0 and B % _XG == 0 and B // _XG == 4 and NG >= 2
    assert Sk % Dh == 0 and M % _SLAB == 0 and D % (16 * _OP_CHUNKS) == 0 and H >= 3
    logB = B.bit_length() - 1
    scale = (Dh ** -0.5) * math.log2(math.e)
    cp = pltpu.make_async_copy

    class Copies:
        def __init__(self, cps):
            self.cps = cps

        def start(self):
            for c in self.cps:
                c.start()

        def wait(self):
            for c in self.cps:
                c.wait()

    def clamp(g):
        return min(g, H - 1) if isinstance(g, int) else jnp.minimum(g, H - 1)

    def x_cp(b):
        return cp(xT_hbm.at[b], xT_buf.at[b], x_sem.at[b])

    def wq_cp(g):
        return Copies([cp(wq_hbm.at[:, pl.ds((clamp(g) * rep + r) * Dh, Dh)], wq_buf.at[g, r], wq_sem.at[g])
                       for r in range(rep)])

    def wo_cp(g):
        return Copies([cp(woT_hbm.at[:, pl.ds((g * rep + r) * Dh, Dh)], wo_buf.at[g, r], wo_sem.at[g])
                       for r in range(rep)])

    def k_last(g):
        return cp(k_hbm.at[0, clamp(g + 1)], k_buf.at[g % 2, B - 1], k_sem.at[g % 2, B - 1])

    def k_rest(g):
        return cp(k_hbm.at[pl.ds(1, B - 1), g], k_buf.at[g % 2, pl.ds(0, B - 1)], k_sem.at[g % 2, 0])

    def v_all(g):
        return cp(v_hbm.at[:, g], v_buf.at[g % 2], v_sem.at[g % 2, 0])

    def group_start(j0):
        for jj in range(_US):
            t1 = j0 + (jj + 1)
            cp(k_hbm.at[t1 & (B - 1), t1 >> logB], k_buf.at[0, j0 + jj], k_sem.at[0, j0]).start()
            cp(v_hbm.at[j0 + jj, 0], v_buf.at[0, j0 + jj], v_sem.at[0, j0]).start()

    def group_wait(j0):
        kb, vb = k_buf.at[0, pl.ds(j0, _US)], v_buf.at[0, pl.ds(j0, _US)]
        cp(kb, kb, k_sem.at[0, j0]).wait()
        cp(vb, vb, v_sem.at[0, j0]).wait()

    def o_cp(b):
        return cp(ostage.at[b], o_hbm.at[b], o_sem.at[0])

    def ld(ref, idx, r0, n, cols=None):
        v = ref.bitcast(i32)[idx + (slice(r0 // 2, (r0 + n) // 2), slice(None) if cols is None else slice(0, cols))]
        return pltpu.bitcast(v, bf16)

    def transpose_x(b):
        for c in range(NC):
            w = min(Dh, D - c * Dh)
            x_buf[b, c, :, 0:w] = ld(xT_buf, (b,), c * Dh, w).T

    def q_proj(g, b):
        xs = jnp.concatenate([ld(x_buf, (b, c), 0, Sq, min(Dh, D - c * Dh)) for c in range(NC)], axis=1)
        for r in range(rep):
            q = jnp.dot(xs, ld(wq_buf, (g, r), 0, D), preferred_element_type=f32)
            q_buf[b, r * Sq:(r + 1) * Sq, :] = (q * scale).astype(bf16)

    def qk(g, j, b):
        return lax.dot_general(ld(q_buf, (b,), 0, M), ld(k_buf, (g % 2, j), 0, Sk), _NT,
                               preferred_element_type=f32)

    def softmax(s_all, par):
        for i in range(M // _SLAB):
            rows = slice(i * _SLAB, (i + 1) * _SLAB)
            s = s_all[rows, :]
            p = jnp.exp2(s - jnp.max(s, axis=-1, keepdims=True))
            l = jnp.sum(p, axis=-1, keepdims=True)
            for c in range(Sk // Dh):
                p_buf[par, c, rows, :] = p[:, c * Dh:(c + 1) * Dh].astype(bf16)
            r = pl.reciprocal(l, approx=True)
            r = r * (2.0 - l * r)
            l_buf[par, rows, :] = jnp.broadcast_to(r, (_SLAB, Dh))

    def pv(g, j, par):
        p = jnp.concatenate([ld(p_buf, (par, c), 0, M) for c in range(Sk // Dh)], axis=1)
        o = jnp.dot(p, ld(v_buf, (g % 2, j), 0, Sk), preferred_element_type=f32)
        o_buf[par] = (o * l_buf[par]).astype(bf16)

    def out_proj(g, b, par, final):
        oc = jnp.concatenate([ld(o_buf, (par,), r * Sq, Sq) for r in range(rep)], axis=1)
        for c in range(0, D, OC):
            w = jnp.concatenate([ld(wo_buf, (g, r), c, OC) for r in range(rep)], axis=1)
            y = lax.dot_general(w, oc, _NT, preferred_element_type=f32)
            if final:
                ostage[b, c:c + OC, :] = (acc[b, c:c + OC, :] + y).astype(bf16)
            else:
                acc[b, c:c + OC, :] += y

    def step(g, j, jj, last=False):
        dyn = not isinstance(j, int)
        if last and j == B - 1:
            s = None
        elif dyn:
            s = qk(g, j, jnp.where(j == B - 1, 0, j + 1) if jj == _US - 1 else j + 1)
        else:
            s = qk(g, j, (j + 1) % B)
        pv(g, j, jj % 2)
        if s is not None:
            softmax(s, (jj + 1) % 2)
        if jj > 0:
            out_proj(g, j - 1, (jj - 1) % 2, last)
        elif dyn:
            out_proj(g, jnp.where(j == 0, B - 1, j - 1), 1, False)
        else:
            out_proj(g - 1, B - 1, 1, False)
        if not last:
            q_proj(g + 1, j)

    def wait_set(g):
        k_rest(g).wait()
        v_all(g).wait()
        wo_cp(g).wait()
        k_last(g).wait()
        wq_cp(g + 1).wait()

    def start_set(g):
        k_rest(g).start()
        v_all(g).start()
        wo_cp(g).start()
        k_last(g).start()
        wq_cp(g + 1).start()

    k00 = cp(k_hbm.at[0, 0], k_buf.at[1, B - 1], k_sem.at[1, B - 1])
    wq_cp(0).start()
    k00.start()
    for b in range(2 * _XG):
        x_cp(b).start()
    zero = jnp.zeros((OC, Sq), f32)
    for b in range(B):
        for c in range(0, D, OC):
            acc[b, c:c + OC, :] = zero
    o_buf[...] = jnp.zeros(o_buf.shape, bf16)
    wq_cp(0).wait()
    for xg in range(B // _XG):
        bs = range(xg * _XG, (xg + 1) * _XG)
        for b in bs:
            x_cp(b).wait()
        if xg + 2 < B // _XG:
            for b in bs:
                x_cp(b + 2 * _XG).start()
        if xg == 0:
            group_start(0)
        elif xg == 1:
            wq_cp(1).start()
            wo_cp(0).start()
        elif xg == 3:
            group_start(_US)
        for b in bs:
            transpose_x(b)
        for b in bs:
            q_proj(0, b)
    k00.wait()
    wq_cp(1).wait()
    wo_cp(0).wait()
    for gg in range(2, NG):
        group_start(gg * _US)
    softmax(qk(-1, B - 1, 0), 0)

    start_set(1)

    def startup_body(i, carry):
        j0 = i * _US
        group_wait(j0)
        for jj in range(_US):
            step(0, j0 + jj, jj)
        return carry

    lax.fori_loop(0, NG, startup_body, 0)

    def main_body(g, carry):
        wait_set(g)
        start_set(g + 1)
        for j in range(B):
            step(g, j, j)
        return carry

    lax.fori_loop(1, H - 1, main_body, 0)

    g = H - 1
    wait_set(g)
    lo = 0
    for j in range(B):
        if j in _GOUT:
            for b in range(lo, j - 1):
                o_cp(b).start()
            lo = j - 1
        step(g, j, j, last=True)
    out_proj(g, B - 1, 1, True)
    for b in range(lo, B):
        o_cp(b).start()
    cp(ostage, o_hbm, o_sem.at[0]).wait()


@jax.jit
def pallas_standalone__gqa_block_cached__near_ridge_kernel(
    x: jax.Array,
    k_cache: jax.Array,
    v_cache: jax.Array,
    wq: jax.Array,
    wo: jax.Array,
):
    bf16, f32 = jnp.bfloat16, jnp.float32
    B, Sq, D = x.shape
    _, H, Sk, Dh = k_cache.shape
    rep = wq.shape[1] // Dh // H
    M = rep * Sq
    hbm = pl.BlockSpec(memory_space=pl.ANY)
    vmem, dma = pltpu.VMEM, pltpu.SemaphoreType.DMA
    outT = pl.pallas_call(
        _kernel,
        in_specs=[hbm] * 5,
        out_specs=hbm,
        out_shape=jax.ShapeDtypeStruct((B, D, Sq), x.dtype),
        scratch_shapes=[
            vmem((B, D, Sq), bf16),
            vmem((B, pl.cdiv(D, Dh), Sq, Dh), bf16),
            vmem((H + 1, rep, D, Dh), bf16),
            vmem((H, rep, D, Dh), bf16),
            vmem((2, B, Sk, Dh), bf16),
            vmem((2, B, Sk, Dh), bf16),
            vmem((B, M, Dh), bf16),
            vmem((2, Sk // Dh, M, Dh), bf16),
            vmem((2, M, Dh), f32),
            vmem((2, M, Dh), bf16),
            vmem((B, D, Sq), f32),
            vmem((B, D, Sq), bf16),
            dma((B,)), dma((H + 1,)), dma((H,)), dma((2, B)), dma((2, B)), dma((1,)),
        ],
        compiler_params=pltpu.CompilerParams(vmem_limit_bytes=100 * 1024 * 1024),
    )(x.transpose(0, 2, 1), k_cache, v_cache, wq, wo.T)
    return outT.transpose(0, 2, 1)
```
